```python
import os as _os
_os.environ.setdefault("JAX_PLATFORMS", "cpu")
import jax
import jax.numpy as jnp

def _softmax(x, axis=-1):
    return jax.nn.softmax(x, axis=axis)
def _gelu(x):
    return jax.nn.gelu(x, approximate=True)
def _silu(x):
    return jax.nn.silu(x)
def _sigmoid(x):
    return jax.nn.sigmoid(x)
def _layernorm(x, axis=-1, eps=1e-5):
    m = jnp.mean(x, axis=axis, keepdims=True)
    v = jnp.var(x, axis=axis, keepdims=True)
    return (x - m) / jnp.sqrt(v + eps)
def _scatter_add(tgt, idx, src, axis=0):
    return tgt.at[idx].add(src)
def _segment_sum(src, seg, n):
    return jax.ops.segment_sum(src, seg, n)
class _Rng:
    def __init__(self, key):
        self._k = key
    def _next(self):
        self._k, sub = jax.random.split(self._k)
        return sub
    def normal(self, shape):
        return jax.random.normal(self._next(), shape, dtype=jnp.bfloat16)
    def randint(self, lo, hi, shape):
        return jax.random.randint(self._next(), shape, lo, hi, dtype=jnp.int32)
    def uniform(self, shape, lo=0.0, hi=1.0):
        return jax.random.uniform(self._next(), shape, jnp.bfloat16, lo, hi)
    def permutation(self, n):
        return jax.random.permutation(self._next(), n)


kernel_name = 'concat_heads__grouped_kv_mqa__sliding_block__prompt'

def setup_inputs():
    _rng = _Rng(jax.random.key(int.from_bytes(__import__("os").urandom(4), "little")))
    _w = (lambda a: (lambda t: t.astype(jnp.bfloat16) if jnp.issubdtype(t.dtype, jnp.floating) else t)(jnp.asarray(a)))
    def _A_setup():
        B, S, D, H = 1, 2048, 1024, 32
        Dh = D // H
        return {
            "x": _w((lambda *s: _rng.normal(s) * 0.05)(B, S, D)),
            "wq": _w((lambda *s: _rng.normal(s) * 1.6)(D, H * Dh)),
            "wk": _w((lambda *s: _rng.normal(s) * 1.6)(D, Dh)),
            "wv": _w((lambda *s: _rng.normal(s) * 0.1)(D, Dh)),
            "wo": _w((lambda *s: _rng.normal(s) * 0.1)(H * Dh, D)),
        }
    _A_in = _A_setup()

    def _B_setup():
        B, S, D = 1, 2048, 1024
        return {
            "x": _w((lambda *s: _rng.normal(s) * 0.2)(B, S, D)),
            "wqkv": _w((lambda *s: _rng.normal(s) * 0.2)(D, 3 * D)),
            "wo": _w((lambda *s: _rng.normal(s) * 0.05)(D, D)),
        }
    _B_in = _B_setup()

    return {
        "A_x": _A_in["x"],
        "A_wq": _A_in["wq"],
        "A_wk": _A_in["wk"],
        "A_wv": _A_in["wv"],
        "A_wo": _A_in["wo"],
        "B_x": _B_in["x"],
        "B_wqkv": _B_in["wqkv"],
        "B_wo": _B_in["wo"],
    }

def reference(A_x, A_wq, A_wk, A_wv, A_wo, B_x, B_wqkv, B_wo):
    def _A_ref(x, wq, wk, wv, wo):
        B, S, D = x.shape
        H = 32
        Dh = D // H
        q = (lambda x, *d: x.transpose(*d))((x @ wq).reshape(B, S, H, Dh), 0, 2, 1, 3)
        k = x @ wk
        v = x @ wv
        scores = jnp.einsum("bhqd,bkd->bhqk", q, k) * (Dh ** -0.5)
        p = _softmax(scores, axis=-1)
        o = jnp.einsum("bhqk,bkd->bhqd", p, v)
        return (lambda x, *d: x.transpose(*d))(o, 0, 2, 1, 3).reshape(B, S, H * Dh) @ wo

    def _B_ref(x, wqkv, wo):
        B, S, D = x.shape
        H = 32; Dh = D // H; W = 256
        qkv = (lambda x, *d: x.transpose(*d))((x @ wqkv).reshape(B, S, 3, H, Dh), 2, 0, 3, 1, 4)
        q, k, v = qkv[0], qkv[1], qkv[2]
        scores = jnp.einsum("bhqd,bhkd->bhqk", q, k) * (Dh ** -0.5)
        idx = jnp.arange(S)
        mask = (idx[:, None] - idx[None, :] >= 0) & (idx[:, None] - idx[None, :] < W)
        scores = jnp.where(mask[None, None], scores, -1e9)
        p = _softmax(scores, axis=-1)
        o = jnp.einsum("bhqk,bhkd->bhqd", p, v)
        return (lambda x, *d: x.transpose(*d))(o, 0, 2, 1, 3).reshape(B, S, D) @ wo

    a = _A_ref(A_x, A_wq, A_wk, A_wv, A_wo)
    b = _B_ref(B_x, B_wqkv, B_wo)
    return jnp.concatenate([a, b], axis=-1)
```

```python
import functools

import jax
import jax.numpy as jnp
import numpy as np
from jax import lax
import jax.experimental.pallas as pl
import jax.experimental.pallas.tpu as pltpu

f32 = jnp.float32
bf16 = jnp.bfloat16

S = 2048
D = 1024
DH = 32
NG = 8
NT = S // 128
WIN = 256
BR = 512
NEG = -1e30
QSCALE = float(DH ** -0.5 * np.log2(np.e))

NT_DIMS = (((1,), (1,)), ((), ()))
TN_DIMS = (((0,), (0,)), ((), ()))
TT_DIMS = (((0,), (1,)), ((), ()))

CFG = dict(a_ck=128, a_thr=2, a_steps=2, b_thr=0)


def _head_weights(qt):
    lane_head = lax.broadcasted_iota(jnp.int32, (128, 128), 1) // DH
    zero = jnp.zeros_like(qt)
    return jnp.concatenate([jnp.where(lane_head == j, qt, zero) for j in range(4)], axis=0)


def _colmax8(s):
    return jnp.max(s.reshape(s.shape[0] // 8, 8, s.shape[1]), axis=0)


def _colsum8(s):
    return jnp.sum(s.reshape(s.shape[0] // 8, 8, s.shape[1]), axis=0)


def _kernel(xa_hbm, wq_hbm, wk_hbm, wv_hbm, woa_hbm, xb_hbm, wqkv_hbm, wob_hbm, out_hbm,
            xa, wq, wk, wv, woa, xb, wqkv, wob,
            qs, k4, vta, ot, kb, vtb, s_a, s_b, bias, ostage, in_sem, out_sem, *, cfg):
    NXA = S // BR
    cp_xa = [pltpu.make_async_copy(xa_hbm.at[0, pl.ds(r * BR, BR), :], xa.at[pl.ds(r * BR, BR), :], in_sem.at[r])
             for r in range(NXA)]
    cp_wq = pltpu.make_async_copy(wq_hbm, wq, in_sem.at[NXA + 0])
    cp_wk = pltpu.make_async_copy(wk_hbm, wk, in_sem.at[NXA + 1])
    cp_wv = pltpu.make_async_copy(wv_hbm, wv, in_sem.at[NXA + 2])
    cp_woa = pltpu.make_async_copy(woa_hbm, woa, in_sem.at[NXA + 3])
    cp_xb = pltpu.make_async_copy(xb_hbm.at[0], xb, in_sem.at[NXA + 4])
    cp_wqkv = pltpu.make_async_copy(wqkv_hbm, wqkv, in_sem.at[NXA + 5])
    cp_wob = pltpu.make_async_copy(wob_hbm, wob, in_sem.at[NXA + 6])

    cp_wq.start()
    cp_xa[0].start()
    cp_wk.start()
    cp_wv.start()
    for r in range(1, NXA):
        cp_xa[r].start()

    kk = lax.broadcasted_iota(jnp.int32, (384, 128), 0)
    qq = lax.broadcasted_iota(jnp.int32, (384, 128), 1)
    for v in range(3):
        dist = (qq + 128 * v) - kk
        bias[v] = jnp.where((dist >= 0) & (dist < WIN), 0.0, NEG).astype(f32)

    cp_wq.wait()
    for r in range(NXA):
        cp_xa[r].wait()
        rows = pl.ds(r * BR, BR)
        q = jnp.dot(xa[rows, :], wq[...], preferred_element_type=f32)
        qs[rows, :] = (q * QSCALE).astype(bf16)
        if r == 0:
            cp_woa.start()
            cp_xb.start()
            cp_wqkv.start()
            cp_wob.start()
    cp_wk.wait()
    cp_wv.wait()
    kt = lax.dot_general(wk[...], xa[...], TT_DIMS, preferred_element_type=f32)
    vt = lax.dot_general(wv[...], xa[...], TT_DIMS, preferred_element_type=f32)
    vta[...] = vt.astype(bf16)
    kt = kt.astype(bf16)
    k4[...] = jnp.concatenate([kt, kt, kt, kt], axis=0).T

    CK = cfg["a_ck"]
    NC = S // CK
    NU = NG * NT

    def a_idx(n):
        t = n // NG
        g = n % NG
        return pl.multiple_of(t * 128, 128), pl.multiple_of(g * 128, 128)

    def a_step(n, slot, m, do_qk=True, do_sm=True):
        if do_qk:
            tq, gl = a_idx(n + 1)
            w = _head_weights(qs[pl.ds(tq, 128), pl.ds(gl, 128)])
        mrun = l = o = None
        hist = []
        for c in range(NC):
            keys = pl.ds(c * CK, CK)
            hist.append(mrun)
            if do_qk:
                s = lax.dot_general(k4[keys, :], w, NT_DIMS, preferred_element_type=f32)
                s_a[1 - slot, keys, :] = s
                mc = _colmax8(s)
                mrun = mc if mrun is None else jnp.maximum(mrun, mc)
            if do_sm:
                mm = m
                thr = cfg["a_thr"]
                if thr and do_qk and c - thr + 1 >= 1:
                    mm = jnp.maximum(m, jnp.minimum(m, hist[c - thr + 1][0:1, :]))
                p = jnp.exp2(s_a[slot, keys, :] - mm)
                lc = _colsum8(p)
                oc = jnp.dot(vta[:, keys], p.astype(bf16), preferred_element_type=f32)
                l = lc if l is None else l + lc
                o = oc if o is None else o + oc
        if do_sm:
            tq, gl = a_idx(n)
            o = (o * (1.0 / jnp.sum(l, axis=0, keepdims=True))).astype(bf16)
            for j in range(4):
                ot[pl.ds(pl.multiple_of(gl + j * DH, DH), DH), pl.ds(tq, 128)] = o[:, j * 128:(j + 1) * 128]
        return jnp.max(mrun, axis=0, keepdims=True) if do_qk else None

    NS = cfg["a_steps"]
    m = a_step(-1, 1, None, do_sm=False)

    def a_body(i, m):
        n = i * NS
        for k in range(NS):
            m = a_step(n + k, k % 2, m)
        return m

    m = lax.fori_loop(0, NU // NS - 1, a_body, m)
    for k in range(NS - 1):
        m = a_step(NU - NS + k, k % 2, m)
    a_step(NU - 1, 1, m, do_qk=False)

    NO = S // BR

    def out_copy(part, r):
        return pltpu.make_async_copy(ostage.at[part * NO + r],
                                     out_hbm.at[0, pl.ds(r * BR, BR), pl.ds(part * D, D)],
                                     out_sem.at[part * NO + r])

    def out_proj(part, wo):
        for r in range(NO):
            y = lax.dot_general(ot[:, pl.ds(r * BR, BR)], wo[...], TN_DIMS, preferred_element_type=f32)
            ostage[part * NO + r] = y.astype(bf16)
            out_copy(part, r).start()

    cp_woa.wait()
    out_proj(0, woa)

    cp_xb.wait()
    cp_wqkv.wait()

    def b_proj(r, c):
        rows = pl.ds(pl.multiple_of(r * BR, BR), BR)
        x = xb[rows, :]
        q = jnp.dot(x, wqkv[:, 0:D], preferred_element_type=f32)
        qs[rows, :] = (q * QSCALE).astype(bf16)
        k = jnp.dot(x, wqkv[:, D:2 * D], preferred_element_type=f32)
        kb[rows, :] = k.astype(bf16)
        v = jnp.dot(x, wqkv[:, 2 * D:3 * D], preferred_element_type=f32)
        vtb[:, rows] = v.astype(bf16).T
        return c

    lax.fori_loop(0, S // BR, b_proj, 0)

    def b_step(t, g, tn, gn, slot, m, do_qk=True, do_sm=True):
        if do_qk:
            tq = pl.multiple_of(tn * 128, 128)
            k0 = pl.multiple_of(jnp.maximum(tn * 128 - WIN, 0), 128)
            vsel = jnp.minimum(tn, 2)
            w = _head_weights(qs[pl.ds(tq, 128), gn * 128:(gn + 1) * 128])
        if do_sm:
            tq_s = pl.multiple_of(t * 128, 128)
            k0_s = pl.multiple_of(jnp.maximum(t * 128 - WIN, 0), 128)
        mrun = l = None
        o = [None] * 4
        hist = []
        for c in range(3):
            hist.append(mrun)
            if do_qk:
                s = lax.dot_general(kb[pl.ds(k0 + c * 128, 128), gn * 128:(gn + 1) * 128], w, NT_DIMS,
                                    preferred_element_type=f32)
                b = bias[vsel, c * 128:(c + 1) * 128, :]
                s = s + jnp.concatenate([b, b, b, b], axis=1)
                s_b[1 - slot, c * 128:(c + 1) * 128, :] = s
                mc = _colmax8(s)
                mrun = mc if mrun is None else jnp.maximum(mrun, mc)
            if do_sm:
                mm = m
                thr = cfg["b_thr"]
                if thr and do_qk and c - thr + 1 >= 1:
                    mm = jnp.maximum(m, jnp.minimum(m, hist[c - thr + 1][0:1, :]))
                p = jnp.exp2(s_b[slot, c * 128:(c + 1) * 128, :] - mm)
                lc = _colsum8(p)
                l = lc if l is None else l + lc
                pb = p.astype(bf16)
                for j in range(4):
                    h = g * 4 + j
                    oc = jnp.dot(vtb[h * DH:(h + 1) * DH, pl.ds(k0_s + c * 128, 128)],
                                 pb[:, j * 128:(j + 1) * 128], preferred_element_type=f32)
                    o[j] = oc if o[j] is None else o[j] + oc
        if do_sm:
            rl = 1.0 / jnp.sum(l, axis=0, keepdims=True)
            for j in range(4):
                h = g * 4 + j
                ot[h * DH:(h + 1) * DH, pl.ds(tq_s, 128)] = (o[j] * rl[:, j * 128:(j + 1) * 128]).astype(bf16)
        return jnp.max(mrun, axis=0, keepdims=True) if do_qk else None

    m = b_step(0, -1, 0, 0, 1, None, do_sm=False)

    def b_body(t, m):
        for g in range(NG):
            if g < NG - 1:
                m = b_step(t, g, t, g + 1, g % 2, m)
            else:
                m = b_step(t, g, jnp.minimum(t + 1, NT - 1), 0, g % 2, m)
        return m

    m = lax.fori_loop(0, NT, b_body, m)

    cp_wob.wait()
    out_proj(1, wob)
    for part in range(2):
        for r in range(NO):
            out_copy(part, r).wait()


def build(cfg, flags=None, name=None):
    def call(A_x, A_wq, A_wk, A_wv, A_wo, B_x, B_wqkv, B_wo):
        any_spec = pl.BlockSpec(memory_space=pl.ANY)
        vmem = pltpu.VMEM
        return pl.pallas_call(
            functools.partial(_kernel, cfg=cfg),
            in_specs=[any_spec] * 8,
            out_specs=any_spec,
            out_shape=jax.ShapeDtypeStruct((1, S, 2 * D), bf16),
            scratch_shapes=[
                vmem((S, D), bf16), vmem((D, D), bf16), vmem((D, DH), bf16), vmem((D, DH), bf16), vmem((D, D), bf16),
                vmem((S, D), bf16), vmem((D, 3 * D), bf16), vmem((D, D), bf16),
                vmem((S, D), bf16),
                vmem((S, 128), bf16),
                vmem((DH, S), bf16),
                vmem((D, S), bf16),
                vmem((S, D), bf16),
                vmem((D, S), bf16),
                vmem((2, S, 512), f32),
                vmem((2, 384, 512), f32),
                vmem((3, 384, 128), f32),
                vmem((2 * S // BR, BR, D), bf16),
                pltpu.SemaphoreType.DMA((S // BR + 7,)),
                pltpu.SemaphoreType.DMA((2 * S // BR,)),
            ],
            compiler_params=pltpu.CompilerParams(vmem_limit_bytes=100 * 2**20, flags=flags),
            name=name,
        )(A_x, A_wq, A_wk, A_wv, A_wo, B_x, B_wqkv, B_wo)
    return call


@jax.jit
def pallas_concat_heads__grouped_kv_mqa__sliding_block__prompt_kernel(
    A_x: jax.Array,
    A_wq: jax.Array,
    A_wk: jax.Array,
    A_wv: jax.Array,
    A_wo: jax.Array,
    B_x: jax.Array,
    B_wqkv: jax.Array,
    B_wo: jax.Array,
):
    return build(CFG)(A_x, A_wq, A_wk, A_wv, A_wo, B_x, B_wqkv, B_wo)
```

```python
import contextlib
import functools

import jax
import jax.numpy as jnp
import numpy as np
from jax import lax
import jax.experimental.pallas as pl
import jax.experimental.pallas.tpu as pltpu

f32 = jnp.float32
bf16 = jnp.bfloat16

S = 2048
D = 1024
DH = 32
NG = 8
NT = S // 128
WIN = 256
BR = 512
NEG = -1e30
MASKED = float(-1e9 * np.log2(np.e))
L_MAX = 2.0 ** 100
V_MAX = 2.0 ** 20
QSCALE = float(DH ** -0.5 * np.log2(np.e))

NT_DIMS = (((1,), (1,)), ((), ()))
TN_DIMS = (((0,), (0,)), ((), ()))

CFG = dict(a_steps=4, lag=2, a_ppos=8, b_ppos=1, b_unroll=2)


def _scope(cfg, name):
    return jax.named_scope(name) if cfg.get("scopes") else contextlib.nullcontext()


def _colmax8(s):
    return jnp.max(s.reshape(s.shape[0] // 8, 8, s.shape[1]), axis=0)


def _colsum8(s):
    return jnp.sum(s.reshape(s.shape[0] // 8, 8, s.shape[1]), axis=0)


def _order_after(m, dep):
    return jnp.maximum(m, jnp.minimum(m, dep[0:1, :]))


def _kernel(xa_hbm, wq_hbm, wkt_hbm, wvt_hbm, woa_hbm, xb_hbm, wqkv_hbm, wob_hbm, out_hbm,
            xa, wq, wkt, wvt, woa, xb, wqkv, wob,
            qt, kpad, vta, ot, kb, vtb, s0, s_x, bias, ostage, in_sem, out_sem, *, cfg):
    NXA = S // BR
    NWQ = 4
    WQC = D // NWQ
    cp_xa = [pltpu.make_async_copy(xa_hbm.at[0, pl.ds(r * BR, BR), :], xa.at[pl.ds(r * BR, BR), :], in_sem.at[r])
             for r in range(NXA)]
    cp_wq = [pltpu.make_async_copy(wq_hbm.at[:, pl.ds(c * WQC, WQC)], wq.at[:, pl.ds(c * WQC, WQC)],
                                   in_sem.at[NXA + c]) for c in range(NWQ)]
    o = NXA + NWQ
    cp_wk = pltpu.make_async_copy(wkt_hbm, wkt, in_sem.at[o + 0])
    cp_wv = pltpu.make_async_copy(wvt_hbm, wvt, in_sem.at[o + 1])
    cp_woa = pltpu.make_async_copy(woa_hbm, woa, in_sem.at[o + 2])
    cp_xb = pltpu.make_async_copy(xb_hbm.at[0], xb, in_sem.at[o + 3])
    cp_wqkv = pltpu.make_async_copy(wqkv_hbm, wqkv, in_sem.at[o + 4])
    cp_wob = pltpu.make_async_copy(wob_hbm, wob, in_sem.at[o + 5])

    cp_xa[0].start()
    for c in range(NWQ):
        cp_wq[c].start()
    cp_wk.start()
    cp_wv.start()
    for r in range(1, NXA):
        cp_xa[r].start()

    kk = lax.broadcasted_iota(jnp.int32, (128, 128), 0)
    qq = lax.broadcasted_iota(jnp.int32, (128, 128), 1)
    bias[0] = jnp.where(kk > qq, 0.0, NEG).astype(f32)
    bias[1] = jnp.where(kk <= qq, 0.0, NEG).astype(f32)

    with _scope(cfg, "p0_aproj"):
        for r in range(NXA):
            cp_xa[r].wait()
            rows = pl.ds(r * BR, BR)
            x = xa[rows, :]
            if r == 0:
                for c in range(NWQ):
                    cp_wq[c].wait()
                    cols = pl.ds(c * WQC, WQC)
                    q = jnp.dot(x, wq[:, cols], preferred_element_type=f32)
                    qt[cols, rows] = (q * QSCALE).astype(bf16).T
                cp_woa.start()
                cp_xb.start()
                cp_wqkv.start()
                cp_wob.start()
                cp_wk.wait()
                cp_wv.wait()
            else:
                q = jnp.dot(x, wq[...], preferred_element_type=f32)
                qt[:, rows] = (q * QSCALE).astype(bf16).T
            kv = lax.dot_general(jnp.concatenate([wkt[...], wvt[...]], axis=0), x, NT_DIMS,
                                 preferred_element_type=f32).astype(bf16)
            kp = jnp.concatenate([kv[:DH, :], jnp.zeros((128 - DH, BR), bf16)], axis=0).T
            if cfg.get("u32"):
                vta[:, rows] = pltpu.bitcast(kv[DH:, :], jnp.uint32)
                kpad[pl.ds(r * BR // 2, BR // 2), :] = pltpu.bitcast(kp, jnp.uint32)
            else:
                vta[:, rows] = kv[DH:, :]
                kpad[rows, :] = kp

    L = cfg["lag"]

    def stream(units, m, chk, probe_next):
        items = [(k, c) for k, u in enumerate(units) for c in range(len(u["chunks"]))]
        ms = {0: m}
        ws, sv, l, o = {}, {}, {}, {}
        for i in range(len(items) + L):
            if i < len(items):
                k, c = items[i]
                u = units[k]
                if c > 0:
                    if k not in ws:
                        ws[k] = u["w"]()
                    sv[(k, c)] = u["chunks"][c]["qk"](ws[k])
                if c == u["ppos"]:
                    nxt = units[k + 1] if k + 1 < len(units) else probe_next
                    if nxt is not None:
                        ms[k + 1] = probe(nxt)
            if i >= L:
                k, c = items[i - L]
                u = units[k]
                ch = u["chunks"][c]
                s = s0[u["slot"]] if c == 0 else sv.pop((k, c))
                p = jnp.exp2(s - ms[k])
                lc = _colsum8(p)
                l[k] = lc if c == 0 else l[k] + lc
                oc = [jnp.dot(ch["v"](jh), p[:, jh * 128:(jh + 1) * 128].astype(bf16), preferred_element_type=f32)
                      for jh in range(4)]
                o[k] = oc if c == 0 else [a + b for a, b in zip(o[k], oc)]
                if c == len(u["chunks"]) - 1:
                    lt = jnp.sum(l.pop(k), axis=0, keepdims=True)
                    rl = 1.0 / lt
                    ok = o.pop(k)
                    for jh in range(4):
                        u["out"](jh, (ok[jh] * rl[:, jh * 128:(jh + 1) * 128]).astype(bf16))
                    chk = jnp.where(lt <= cfg.get("l_max", L_MAX), chk, 1.0)
        return ms.get(len(units)), chk

    def probe(u):
        s = u["chunks"][0]["qk"](u["w"]())
        s0[u["slot"]] = s
        return jnp.max(_colmax8(s), axis=0, keepdims=True)

    def exact_quad(w, nchunk, qk, vth, out):
        def pass1(c, mrun):
            s = qk(w, c)
            s_x[pl.ds(pl.multiple_of(c * 128, 128), 128), :] = s
            return jnp.maximum(mrun, _colmax8(s))
        m = jnp.max(lax.fori_loop(0, nchunk, pass1, jnp.full((8, 512), -jnp.inf, f32)), axis=0, keepdims=True)

        def pass2(c, carry):
            l, o = carry
            p = jnp.exp2(s_x[pl.ds(pl.multiple_of(c * 128, 128), 128), :] - m)
            oc = jnp.concatenate(
                [jnp.dot(vth(c, jh), p[:, jh * 128:(jh + 1) * 128].astype(bf16), preferred_element_type=f32)
                 for jh in range(4)], axis=1)
            return l + _colsum8(p), o + oc
        l, o = lax.fori_loop(0, nchunk, pass2, (jnp.zeros((8, 512), f32), jnp.zeros((DH, 512), f32)))
        o = o * (1.0 / jnp.sum(l, axis=0, keepdims=True))
        for jh in range(4):
            out(jh, o[:, jh * 128:(jh + 1) * 128].astype(bf16))

    def raised(chk, v_ref):
        v_ok = jnp.max(jnp.abs(v_ref[...].astype(f32))) <= V_MAX
        return jnp.logical_or(jnp.max(chk) > 0.0, jnp.logical_not(v_ok))

    NU = NG * NT
    zpad = jnp.zeros((128 - DH, 128), bf16)

    def a_idx(n):
        return pl.multiple_of((n // NG) * 128, 128), pl.multiple_of((n % NG) * 128, 128)

    def a_w(n):
        tq, gl = a_idx(n)
        return jnp.concatenate(
            [jnp.concatenate([qt[pl.ds(pl.multiple_of(gl + j * DH, DH), DH), pl.ds(tq, 128)], zpad], axis=0)
             for j in range(4)], axis=1)

    def a_out(n, jh, val):
        tq, gl = a_idx(n)
        ot[pl.ds(pl.multiple_of(gl + jh * DH, DH), DH), pl.ds(tq, 128)] = val

    def a_unit(n, slot):
        def chunk(c):
            return dict(qk=lambda w: jnp.dot(kpad[c * 128:(c + 1) * 128, :], w, preferred_element_type=f32),
                        v=lambda jh: vta[:, c * 128:(c + 1) * 128])
        return dict(w=lambda: a_w(n), chunks=[chunk(c) for c in range(S // 128)], slot=slot,
                    ppos=cfg["a_ppos"], out=functools.partial(a_out, n))

    NS = cfg["a_steps"]
    chk0 = jnp.zeros((1, 512), f32)
    with _scope(cfg, "p1_aattn"):
        m = probe(a_unit(0, 0))

        def a_body(i, carry):
            n = i * NS
            return stream([a_unit(n + k, k % 2) for k in range(NS)], carry[0], carry[1], a_unit(n + NS, 0))

        m, chk = lax.fori_loop(0, NU // NS - 1, a_body, (m, chk0))
        _, chk = stream([a_unit(NU - NS + k, k % 2) for k in range(NS)], m, chk, None)

        @pl.when(raised(chk, vta))
        def _():
            def body(n, c):
                exact_quad(
                    a_w(n), S // 128,
                    lambda w, c: jnp.dot(kpad[pl.ds(pl.multiple_of(c * 128, 128), 128), :], w,
                                         preferred_element_type=f32),
                    lambda c, jh: vta[:, pl.ds(pl.multiple_of(c * 128, 128), 128)],
                    functools.partial(a_out, n))
                return c
            lax.fori_loop(0, NU, body, 0)

    OB = cfg.get("o_blocks", (512, 512, 512, 256, 256))
    OO = [sum(OB[:i]) for i in range(len(OB))]
    NO = len(OB)

    def out_copy(part, r):
        return pltpu.make_async_copy(ostage.at[part, pl.ds(OO[r], OB[r]), :],
                                     out_hbm.at[0, pl.ds(OO[r], OB[r]), pl.ds(part * D, D)],
                                     out_sem.at[part * NO + r])

    def out_proj(part, wo):
        for r in range(NO):
            y = lax.dot_general(ot[:, pl.ds(OO[r], OB[r])], wo[...], TN_DIMS, preferred_element_type=f32)
            ostage[part, pl.ds(OO[r], OB[r]), :] = y.astype(bf16)
            out_copy(part, r).start()

    with _scope(cfg, "p2_aout"):
        cp_woa.wait()
        out_proj(0, woa)

    with _scope(cfg, "p3_bproj"):
        cp_xb.wait()
        cp_wqkv.wait()

        def b_proj(r, c):
            rows = pl.ds(pl.multiple_of(r * BR, BR), BR)
            x = xb[rows, :]
            q = jnp.dot(x, wqkv[:, 0:D], preferred_element_type=f32)
            qt[:, rows] = (q * QSCALE).astype(bf16).T
            k = jnp.dot(x, wqkv[:, D:2 * D], preferred_element_type=f32)
            kb[rows, :] = k.astype(bf16)
            v = jnp.dot(x, wqkv[:, 2 * D:3 * D], preferred_element_type=f32)
            vtb[:, rows] = v.astype(bf16).T
            return c

        lax.fori_loop(0, S // BR, b_proj, 0)

    def b_w(g, tq):
        ws = []
        for j in range(4):
            parts = [
                qt[g * 128 + j * DH:g * 128 + (j + 1) * DH, pl.ds(tq, 128)]]
            if j > 0:
                parts.insert(0, jnp.zeros((j * DH, 128), bf16))
            if j < 3:
                parts.append(jnp.zeros((128 - (j + 1) * DH, 128), bf16))
            ws.append(jnp.concatenate(parts, axis=0))
        return jnp.concatenate(ws, axis=1)

    def b_unit(t, g, slot):
        static = isinstance(t, int)
        mult = (lambda x: x) if static else (lambda x: pl.multiple_of(x, 128))
        tq = mult(t * 128)
        lanes = slice(g * 128, (g + 1) * 128)

        def chunk(k0, b):
            k0 = mult(k0)

            def qk(w):
                s = jnp.dot(kb[pl.ds(k0, 128), lanes], w, preferred_element_type=f32)
                if b is not None:
                    t_b = bias[b]
                    s = s + jnp.concatenate([t_b] * 4, axis=1)
                return s
            return dict(qk=qk, v=lambda jh: vtb[(g * 4 + jh) * DH:(g * 4 + jh + 1) * DH, pl.ds(k0, 128)])
        if static and t == 0:
            chunks = [chunk(tq, 1)]
        elif static and t == 1:
            chunks = [chunk(tq - 128, None), chunk(tq, 1)]
        else:
            chunks = [chunk(tq - 128, None), chunk(tq - 256, 0), chunk(tq, 1)]

        def out(jh, val):
            ot[(g * 4 + jh) * DH:(g * 4 + jh + 1) * DH, pl.ds(tq, 128)] = val
        return dict(w=lambda: b_w(g, tq), chunks=chunks, slot=slot, ppos=min(cfg["b_ppos"], len(chunks) - 1), out=out)

    with _scope(cfg, "p4_battn"):
        U = cfg["b_unroll"]
        m = probe(b_unit(0, 0, 0))
        two = jnp.int32(2)
        m, chk = stream([b_unit(t, g, g % 4) for t in range(2) for g in range(NG)], m, chk0, b_unit(two, 0, 0))

        def b_body(i, carry):
            t0 = 2 + i * U
            return stream([b_unit(t0 + u, g, g % 4) for u in range(U) for g in range(NG)], carry[0], carry[1],
                          b_unit(t0 + U, 0, 0))

        m, chk = lax.fori_loop(0, (NT - 2) // U - 1, b_body, (m, chk))
        t0 = NT - U
        _, chk = stream([b_unit(t0 + u, g, g % 4) for u in range(U) for g in range(NG)], m, chk, None)

        @pl.when(raised(chk, vtb))
        def _():
            kk = lax.broadcasted_iota(jnp.int32, (128, 512), 0)
            qq = lax.broadcasted_iota(jnp.int32, (128, 512), 1) % 128

            def body(n, c):
                t = n // NG
                gl = pl.multiple_of((n % NG) * 128, 128)
                tq = pl.multiple_of(t * 128, 128)
                k0 = pl.multiple_of(jnp.maximum(tq - WIN, 0), 128)
                w = jnp.concatenate(
                    [jnp.where(lax.broadcasted_iota(jnp.int32, (128, 128), 0) // DH == j,
                               qt[pl.ds(gl, 128), pl.ds(tq, 128)].astype(f32), 0.0).astype(bf16) for j in range(4)],
                    axis=1)

                def qk(w, c):
                    ks = pl.multiple_of(k0 + c * 128, 128)
                    s = jnp.dot(kb[pl.ds(ks, 128), pl.ds(gl, 128)], w, preferred_element_type=f32)
                    dist = (tq + qq) - (ks + kk)
                    return jnp.where((dist >= 0) & (dist < WIN), s, MASKED)

                def out(jh, val):
                    ot[pl.ds(pl.multiple_of(gl + jh * DH, DH), DH), pl.ds(tq, 128)] = val
                exact_quad(
                    w, 3, qk,
                    lambda c, jh: vtb[pl.ds(pl.multiple_of(gl + jh * DH, DH), DH),
                                      pl.ds(pl.multiple_of(k0 + c * 128, 128), 128)],
                    out)
                return c
            lax.fori_loop(0, NU, body, 0)

    with _scope(cfg, "p5_bout"):
        cp_wob.wait()
        out_proj(1, wob)
        for part in range(2):
            for r in range(NO):
                out_copy(part, r).wait()


def build(cfg, flags=None, name=None):
    def call(A_x, A_wq, A_wk, A_wv, A_wo, B_x, B_wqkv, B_wo):
        any_spec = pl.BlockSpec(memory_space=pl.ANY)
        vmem = pltpu.VMEM
        NO = len(cfg.get("o_blocks", (512, 512, 512, 256, 256)))
        return pl.pallas_call(
            functools.partial(_kernel, cfg=cfg),
            in_specs=[any_spec] * 8,
            out_specs=any_spec,
            out_shape=jax.ShapeDtypeStruct((1, S, 2 * D), bf16),
            scratch_shapes=[
                vmem((S, D), bf16), vmem((D, D), bf16), vmem((DH, D), bf16), vmem((DH, D), bf16), vmem((D, D), bf16),
                vmem((S, D), bf16), vmem((D, 3 * D), bf16), vmem((D, D), bf16),
                vmem((D, S), bf16),
                vmem((S // 2, 128), jnp.uint32) if cfg.get("u32") else vmem((S, 128), bf16),
                vmem((DH // 2, S), jnp.uint32) if cfg.get("u32") else vmem((DH, S), bf16),
                vmem((D, S), bf16),
                vmem((S, D), bf16),
                vmem((D, S), bf16),
                vmem((4, 128, 512), f32),
                vmem((S, 512), f32),
                vmem((2, 128, 128), f32),
                vmem((2, S, D), bf16),
                pltpu.SemaphoreType.DMA((S // BR + 4 + 6,)),
                pltpu.SemaphoreType.DMA((2 * NO,)),
            ],
            compiler_params=pltpu.CompilerParams(vmem_limit_bytes=100 * 2**20, flags=flags),
            name=name,
        )(A_x, A_wq, A_wk.T, A_wv.T, A_wo, B_x, B_wqkv, B_wo)
    return call


@jax.jit
def pallas_concat_heads__grouped_kv_mqa__sliding_block__prompt_kernel(
    A_x: jax.Array,
    A_wq: jax.Array,
    A_wk: jax.Array,
    A_wv: jax.Array,
    A_wo: jax.Array,
    B_x: jax.Array,
    B_wqkv: jax.Array,
    B_wo: jax.Array,
):
    return build(CFG)(A_x, A_wq, A_wk, A_wv, A_wo, B_x, B_wqkv, B_wo)
```

```python
import functools

import jax
import jax.numpy as jnp
import numpy as np
from jax import lax
import jax.experimental.pallas as pl
import jax.experimental.pallas.tpu as pltpu

f32 = jnp.float32
bf16 = jnp.bfloat16

S = 2048
D = 1024
DH = 32
NG = D // 128
NT = S // 128
NQ = NG * NT
WIN = 256
BR = 512

LOG2E = float(np.log2(np.e))
QSCALE = DH ** -0.5 * LOG2E
MASKED = -1e9 * LOG2E
L_MAX = 2.0 ** 100
V_MAX = 2.0 ** 20
M_MIN = -1e8

LAG = 1
A_HEAD, A_STEP = 2, 6
B_HEAD, B_STEP = 4, 4
X_BLOCKS = ((0, 256), (256, 256), (512, 512), (1024, 1024))
WQ_BLOCKS = ((0, 256), (256, 256), (512, 512))
OUT_BLOCKS = ((0, 512), (512, 512), (1024, 512), (1536, 256), (1792, 128), (1920, 128))

NT_DIMS = (((1,), (1,)), ((), ()))
TN_DIMS = (((0,), (0,)), ((), ()))


def _dot(a, b):
    return jnp.dot(a, b, preferred_element_type=f32)


def _colmax8(s):
    return jnp.max(s.reshape(s.shape[0] // 8, 8, s.shape[1]), axis=0)


def _colsum8(s):
    return jnp.sum(s.reshape(s.shape[0] // 8, 8, s.shape[1]), axis=0)


def _tile(i):
    return i * 128 if isinstance(i, int) else pl.multiple_of(i * 128, 128)


def _kernel(xa_hbm, wq_hbm, wkt_hbm, wvt_hbm, woa_hbm, xb_hbm, wqkv_hbm, wob_hbm, out_hbm,
            xa, wq, wkt, wvt, woa, xb, wqkv, wob,
            qt, kpad, vta, kb, vtb, ot, s_probe, p_held, s_all, bias, ostage, in_sem, out_sem):
    sems = iter(range(in_sem.shape[0]))
    copy = lambda src, dst: pltpu.make_async_copy(src, dst, in_sem.at[next(sems)])
    cp_x = [copy(xa_hbm.at[0, pl.ds(a, n), :], xa.at[pl.ds(a, n), :]) for a, n in X_BLOCKS]
    cp_wq = [copy(wq_hbm.at[:, pl.ds(a, n)], wq.at[:, pl.ds(a, n)]) for a, n in WQ_BLOCKS]
    cp_wk, cp_wv = copy(wkt_hbm, wkt), copy(wvt_hbm, wvt)
    cp_woa, cp_xb, cp_wqkv, cp_wob = copy(woa_hbm, woa), copy(xb_hbm.at[0], xb), copy(wqkv_hbm, wqkv), copy(wob_hbm, wob)
    for cp in (cp_x[0], cp_wq[0], cp_x[1], cp_wq[1], cp_wq[2], cp_wk, cp_wv, cp_x[2], cp_x[3]):
        cp.start()

    kk = lax.broadcasted_iota(jnp.int32, (128, 128), 0)
    qq = lax.broadcasted_iota(jnp.int32, (128, 128), 1)
    bias[0] = jnp.where(kk > qq, 0.0, -jnp.inf).astype(f32)
    bias[1] = jnp.where(kk <= qq, 0.0, -jnp.inf).astype(f32)

    def a_q(r0, nr, c0, nc):
        rows, cols = pl.ds(r0, nr), pl.ds(c0, nc)
        qt[cols, rows] = (_dot(xa[rows, :], wq[:, cols]) * QSCALE).astype(bf16).T

    def a_kv(r0):
        rows = pl.ds(r0, BR)
        kv = lax.dot_general(jnp.concatenate([wkt[...], wvt[...]], axis=0), xa[rows, :], NT_DIMS,
                             preferred_element_type=f32).astype(bf16)
        vta[:, rows] = kv[DH:, :]
        kpad[rows, :] = jnp.concatenate([kv[:DH, :], jnp.zeros((128 - DH, BR), bf16)], axis=0).T

    cp_x[0].wait()
    cp_wq[0].wait()
    a_q(0, 256, 0, 256)
    cp_x[1].wait()
    a_q(256, 256, 0, 256)
    cp_wq[1].wait()
    a_q(0, 512, 256, 256)
    cp_wq[2].wait()
    a_q(0, 512, 512, 512)
    cp_x[2].wait()
    cp_wk.wait()
    cp_wv.wait()
    a_q(512, 512, 0, D)
    a_kv(0)
    a_kv(512)
    cp_x[3].wait()
    for r0 in (1024, 1536):
        a_q(r0, 512, 0, D)
    for r0 in (1024, 1536):
        a_kv(r0)

    def probe(u):
        s = u["chunks"][0]["qk"](u["w"]())
        s_probe[u["slot"]] = s
        return jnp.max(_colmax8(s), axis=0, keepdims=True)

    def stream(quads, m, bad, after, prev=None, carry=None, hold=False):
        ahead = []
        for k, u in enumerate(quads):
            ahead += [(k, c) for c in range(1, len(u["chunks"]))] + [(k, None)]
        todo = [(k, c) for k, u in enumerate(quads) for c in range(len(u["chunks"]))]
        ms, ws, sv, l, o = {0: m}, {}, {}, {}, {}
        first = LAG
        if prev is not None:
            ms[-1], l[-1], o[-1] = carry
            todo = [(-1, len(prev["chunks"]) - 1)] + todo
            first = LAG - 1
        for i in range(len(todo) + first):
            if i < len(ahead):
                k, c = ahead[i]
                if c is not None:
                    if k not in ws:
                        ws[k] = quads[k]["w"]()
                    sv[(k, c)] = quads[k]["chunks"][c]["qk"](ws[k])
                else:
                    nxt = quads[k + 1] if k + 1 < len(quads) else after
                    if nxt is not None:
                        ms[k + 1] = probe(nxt)
            if i < first:
                continue
            k, c = todo[i - first]
            u = prev if k < 0 else quads[k]
            if k < 0:
                pb = [p_held[j] for j in range(4)]
            else:
                p = jnp.exp2((s_probe[u["slot"]] if c == 0 else sv.pop((k, c))) - ms[k])
                l[k] = _colsum8(p) if c == 0 else l[k] + _colsum8(p)
                pb = [p[:, j * 128:(j + 1) * 128].astype(bf16) for j in range(4)]
                if hold and i - first == len(todo) - 1:
                    for j in range(4):
                        p_held[j] = pb[j]
                    continue
            oc = [_dot(u["chunks"][c]["v"](j), pb[j]) for j in range(4)]
            o[k] = oc if c == 0 else [a + b for a, b in zip(o[k], oc)]
            if c == len(u["chunks"]) - 1:
                lt = jnp.sum(l.pop(k), axis=0, keepdims=True)
                rl = 1.0 / lt
                for j, oj in enumerate(o.pop(k)):
                    u["out"](j, (oj * rl[:, j * 128:(j + 1) * 128]).astype(bf16))
                bad = jnp.where((lt <= L_MAX) & (ms[k] >= M_MIN), bad, 1.0)
        kl = len(quads) - 1
        return ms.get(len(quads)), bad, ((ms[kl], l[kl], o[kl]) if hold else None)

    def redo_with_true_max(bad, v_absmax, n_quad):
        @pl.when(jnp.logical_or(jnp.max(bad) > 0.0, jnp.logical_not(v_absmax <= V_MAX)))
        def _():
            def body(n, carry):
                w, qk, vt, out = n_quad(n)

                def pass1(c, mrun):
                    s = qk(w, _tile(c))
                    s_all[pl.ds(_tile(c), 128), :] = s
                    return jnp.maximum(mrun, _colmax8(s))
                mrun = lax.fori_loop(0, NT, pass1, jnp.full((8, 512), -jnp.inf, f32))
                m = jnp.max(mrun, axis=0, keepdims=True)

                def pass2(c, lo):
                    p = jnp.exp2(s_all[pl.ds(_tile(c), 128), :] - m)
                    oc = jnp.concatenate(
                        [_dot(vt(j, _tile(c)), p[:, j * 128:(j + 1) * 128].astype(bf16)) for j in range(4)], axis=1)
                    return lo[0] + _colsum8(p), lo[1] + oc
                l, o = lax.fori_loop(0, NT, pass2, (jnp.zeros((8, 512), f32), jnp.zeros((DH, 512), f32)))
                o = o * (1.0 / jnp.sum(l, axis=0, keepdims=True))
                for j in range(4):
                    out(j, o[:, j * 128:(j + 1) * 128].astype(bf16))
                return carry
            lax.fori_loop(0, NQ, body, 0)

    def head_rows(gl, j):
        return pl.ds(gl + j * DH if isinstance(gl, int) else pl.multiple_of(gl + j * DH, DH), DH)

    def store_head(gl, tq, j, val):
        ot[head_rows(gl, j), pl.ds(tq, 128)] = val

    def stationary(gl, tq, diagonal):
        blocks = []
        for j in range(4):
            above = j * DH if diagonal else 0
            parts = [jnp.zeros((above, 128), bf16)] if above else []
            parts.append(qt[head_rows(gl, j), pl.ds(tq, 128)])
            if above + DH < 128:
                parts.append(jnp.zeros((128 - above - DH, 128), bf16))
            blocks.append(jnp.concatenate(parts, axis=0))
        return jnp.concatenate(blocks, axis=1)

    no_flag = jnp.zeros((1, 512), f32)

    def a_quad(n, slot):
        tq, gl = _tile(n // NG), _tile(n % NG)

        def chunk(c):
            keys = pl.ds(c * 128, 128)
            return dict(qk=lambda w: _dot(kpad[keys, :], w), v=lambda j: vta[:, keys])
        return dict(w=lambda: stationary(gl, tq, False), chunks=[chunk(c) for c in range(NT)], slot=slot,
                    out=functools.partial(store_head, gl, tq))

    m, bad, held = stream([a_quad(k, k % 2) for k in range(A_HEAD)], probe(a_quad(0, 0)), no_flag,
                          a_quad(A_HEAD, 0), hold=True)
    for cp in (cp_woa, cp_xb, cp_wqkv, cp_wob):
        cp.start()

    def a_trip(i, carry):
        n = A_HEAD + i * A_STEP
        m, bad, held = carry
        return stream([a_quad(n + k, k % 2) for k in range(A_STEP)], m, bad,
                      a_quad(jnp.minimum(n + A_STEP, NQ - 1), 0), prev=a_quad(n - 1, 1), carry=held, hold=True)

    m, bad, held = lax.fori_loop(0, (NQ - A_HEAD) // A_STEP, a_trip, (m, bad, held))
    _, bad, _ = stream([], m, bad, None, prev=a_quad(NQ - 1, 1), carry=held)

    def a_exact(n):
        tq, gl = _tile(n // NG), _tile(n % NG)
        return (stationary(gl, tq, False), lambda w, k0: _dot(kpad[pl.ds(k0, 128), :], w),
                lambda j, k0: vta[:, pl.ds(k0, 128)], functools.partial(store_head, gl, tq))

    redo_with_true_max(bad, jnp.max(jnp.abs(vta[...].astype(f32))), a_exact)

    def out_copy(part, i):
        a, n = OUT_BLOCKS[i]
        return pltpu.make_async_copy(ostage.at[part, pl.ds(a, n), :], out_hbm.at[0, pl.ds(a, n), pl.ds(part * D, D)],
                                     out_sem.at[part * len(OUT_BLOCKS) + i])

    def out_proj(part, wo):
        for i, (a, n) in enumerate(OUT_BLOCKS):
            y = lax.dot_general(ot[:, pl.ds(a, n)], wo[...], TN_DIMS, preferred_element_type=f32)
            ostage[part, pl.ds(a, n), :] = y.astype(bf16)
            out_copy(part, i).start()

    cp_woa.wait()
    cp_xb.wait()
    cp_wqkv.wait()
    cp_wob.wait()
    out_proj(0, woa)

    def b_proj(r, vmax):
        rows = pl.ds(pl.multiple_of(r * BR, BR), BR)
        x = xb[rows, :]
        qt[:, rows] = (_dot(x, wqkv[:, 0:D]) * QSCALE).astype(bf16).T
        kb[rows, :] = _dot(x, wqkv[:, D:2 * D]).astype(bf16)
        v = _dot(x, wqkv[:, 2 * D:3 * D])
        vtb[:, rows] = v.astype(bf16).T
        return jnp.maximum(vmax, _colmax8(jnp.abs(v)))

    vb_absmax = jnp.max(lax.fori_loop(0, S // BR, b_proj, jnp.zeros((8, D), f32)))

    def b_quad(t, g):
        gl, tq = g * 128, _tile(t)

        def chunk(back, mask):
            keys = pl.ds(_tile(t - back), 128)

            def qk(w):
                s = _dot(kb[keys, gl:gl + 128], w)
                return s if mask is None else s + jnp.concatenate([bias[mask]] * 4, axis=1)
            return dict(qk=qk, v=lambda j: vtb[head_rows(gl, j), keys])
        chunks = [chunk(1, None), chunk(2, 0), chunk(0, 1)]
        if isinstance(t, int) and t < 2:
            chunks = chunks[2:] if t == 0 else [chunks[0], chunks[2]]
        return dict(w=lambda: stationary(gl, tq, True), chunks=chunks, slot=g % 4,
                    out=functools.partial(store_head, gl, tq))

    def tiles(ts):
        return [b_quad(t, g) for t in ts for g in range(NG)]

    m, bad, held = stream(tiles(range(B_HEAD)), probe(b_quad(0, 0)), no_flag, b_quad(B_HEAD, 0), hold=True)

    def b_trip(i, carry):
        t = B_HEAD + i * B_STEP
        m, bad, held = carry
        return stream(tiles([t + u for u in range(B_STEP)]), m, bad, b_quad(jnp.minimum(t + B_STEP, NT - 1), 0),
                      prev=b_quad(t - 1, NG - 1), carry=held, hold=True)

    m, bad, held = lax.fori_loop(0, (NT - B_HEAD) // B_STEP, b_trip, (m, bad, held))
    _, bad, _ = stream([], m, bad, None, prev=b_quad(NT - 1, NG - 1), carry=held)

    def b_exact(n):
        tq, gl = _tile(n // NG), _tile(n % NG)
        lane_head = lax.broadcasted_iota(jnp.int32, (128, 128), 0) // DH
        q = qt[pl.ds(gl, 128), pl.ds(tq, 128)].astype(f32)
        w = jnp.concatenate([jnp.where(lane_head == j, q, 0.0).astype(bf16) for j in range(4)], axis=1)
        qpos = tq + lax.broadcasted_iota(jnp.int32, (128, 512), 1) % 128

        def qk(w, k0):
            dist = qpos - (k0 + lax.broadcasted_iota(jnp.int32, (128, 512), 0))
            s = _dot(kb[pl.ds(k0, 128), pl.ds(gl, 128)], w)
            return jnp.where((dist >= 0) & (dist < WIN), s, MASKED)
        return w, qk, lambda j, k0: vtb[head_rows(gl, j), pl.ds(k0, 128)], functools.partial(store_head, gl, tq)

    redo_with_true_max(bad, vb_absmax, b_exact)

    out_proj(1, wob)
    for part in range(2):
        for i in range(len(OUT_BLOCKS)):
            out_copy(part, i).wait()


@jax.jit
def pallas_concat_heads__grouped_kv_mqa__sliding_block__prompt_kernel(
    A_x: jax.Array,
    A_wq: jax.Array,
    A_wk: jax.Array,
    A_wv: jax.Array,
    A_wo: jax.Array,
    B_x: jax.Array,
    B_wqkv: jax.Array,
    B_wo: jax.Array,
):
    hbm = pl.BlockSpec(memory_space=pl.ANY)
    vmem = pltpu.VMEM
    return pl.pallas_call(
        _kernel,
        in_specs=[hbm] * 8,
        out_specs=hbm,
        out_shape=jax.ShapeDtypeStruct((1, S, 2 * D), bf16),
        scratch_shapes=[
            vmem((S, D), bf16), vmem((D, D), bf16), vmem((DH, D), bf16), vmem((DH, D), bf16), vmem((D, D), bf16),
            vmem((S, D), bf16), vmem((D, 3 * D), bf16), vmem((D, D), bf16),
            vmem((D, S), bf16),
            vmem((S, 128), bf16),
            vmem((DH, S), bf16),
            vmem((S, D), bf16),
            vmem((D, S), bf16),
            vmem((D, S), bf16),
            vmem((4, 128, 512), f32),
            vmem((4, 128, 128), bf16),
            vmem((S, 512), f32),
            vmem((2, 128, 128), f32),
            vmem((2, S, D), bf16),
            pltpu.SemaphoreType.DMA((len(X_BLOCKS) + len(WQ_BLOCKS) + 6,)),
            pltpu.SemaphoreType.DMA((2 * len(OUT_BLOCKS),)),
        ],
        compiler_params=pltpu.CompilerParams(vmem_limit_bytes=100 * 2**20),
    )(A_x, A_wq, A_wk.T, A_wv.T, A_wo, B_x, B_wqkv, B_wo)
```

```python
import functools

import jax
import jax.numpy as jnp
import numpy as np
from jax import lax
import jax.experimental.pallas as pl
import jax.experimental.pallas.tpu as pltpu

f32 = jnp.float32
bf16 = jnp.bfloat16

S = 2048
D = 1024
DH = 32
NG = D // 128
NT = S // 128
NQ = NG * NT
WIN = 256
BR = 512

LOG2E = float(np.log2(np.e))
QSCALE = DH ** -0.5 * LOG2E
MASKED = -1e9 * LOG2E
L_MAX = 2.0 ** 100
V_MAX = 2.0 ** 20
M_MIN = -1e8

LAG = 1
A_STEP = 8
X_BLOCKS = ((0, 256), (256, 256), (512, 512), (1024, 1024))
WQ_BLOCKS = ((0, 256), (256, 256), (512, 512))
OUT_BLOCKS = ((0, 512), (512, 512), (1024, 512), (1536, 256), (1792, 128), (1920, 128))

NT_DIMS = (((1,), (1,)), ((), ()))
TN_DIMS = (((0,), (0,)), ((), ()))


def _dot(a, b):
    return jnp.dot(a, b, preferred_element_type=f32)


def _colmax8(s):
    return jnp.max(s.reshape(s.shape[0] // 8, 8, s.shape[1]), axis=0)


def _colsum8(s):
    return jnp.sum(s.reshape(s.shape[0] // 8, 8, s.shape[1]), axis=0)


def _tile(i):
    return i * 128 if isinstance(i, int) else pl.multiple_of(i * 128, 128)


def _kernel(xa_hbm, wq_hbm, wkt_hbm, wvt_hbm, woa_hbm, xb_hbm, wqkv_hbm, wob_hbm, out_hbm,
            xa, wq, wkt, wvt, woa, xb, wqkv, wob,
            qt, kpad, vta, kb, vtb, ot, s_probe, p_held, s_all, bias, ostage, in_sem, out_sem):
    sems = iter(range(in_sem.shape[0]))
    copy = lambda src, dst: pltpu.make_async_copy(src, dst, in_sem.at[next(sems)])
    cp_x = [copy(xa_hbm.at[0, pl.ds(a, n), :], xa.at[pl.ds(a, n), :]) for a, n in X_BLOCKS]
    cp_wq = [copy(wq_hbm.at[:, pl.ds(a, n)], wq.at[:, pl.ds(a, n)]) for a, n in WQ_BLOCKS]
    cp_wk, cp_wv = copy(wkt_hbm, wkt), copy(wvt_hbm, wvt)
    cp_woa, cp_xb, cp_wqkv, cp_wob = copy(woa_hbm, woa), copy(xb_hbm.at[0], xb), copy(wqkv_hbm, wqkv), copy(wob_hbm, wob)
    for cp in (cp_x[0], cp_wq[0], cp_x[1], cp_wq[1], cp_wq[2], cp_wk, cp_wv, cp_x[2], cp_x[3]):
        cp.start()

    kk = lax.broadcasted_iota(jnp.int32, (128, 128), 0)
    qq = lax.broadcasted_iota(jnp.int32, (128, 128), 1)
    bias[0] = jnp.where(kk > qq, 0.0, -jnp.inf).astype(f32)
    bias[1] = jnp.where(kk <= qq, 0.0, -jnp.inf).astype(f32)

    def a_q(r0, nr, c0, nc):
        rows, cols = pl.ds(r0, nr), pl.ds(c0, nc)
        qt[cols, rows] = (_dot(xa[rows, :], wq[:, cols]) * QSCALE).astype(bf16).T

    def a_kv(r0):
        rows = pl.ds(r0, BR)
        kv = lax.dot_general(jnp.concatenate([wkt[...], wvt[...]], axis=0), xa[rows, :], NT_DIMS,
                             preferred_element_type=f32).astype(bf16)
        vta[:, rows] = kv[DH:, :]
        kpad[rows, :] = jnp.concatenate([kv[:DH, :], jnp.zeros((128 - DH, BR), bf16)], axis=0).T

    cp_x[0].wait()
    cp_wq[0].wait()
    a_q(0, 256, 0, 256)
    cp_x[1].wait()
    a_q(256, 256, 0, 256)
    cp_wq[1].wait()
    a_q(0, 512, 256, 256)
    cp_wq[2].wait()
    a_q(0, 512, 512, 512)
    cp_x[2].wait()
    cp_wk.wait()
    cp_wv.wait()
    a_q(512, 512, 0, D)
    a_kv(0)
    a_kv(512)
    cp_x[3].wait()
    for r0 in (1024, 1536):
        a_q(r0, 512, 0, D)
    for r0 in (1024, 1536):
        a_kv(r0)

    def probe(u):
        s = u["chunks"][0]["qk"](u["w"]())
        s_probe[u["slot"]] = s
        return jnp.max(_colmax8(s), axis=0, keepdims=True)

    def stream(quads, m, bad, after, prev=None, carry=None, hold=False):
        ahead = []
        for k, u in enumerate(quads):
            ahead += [(k, c) for c in range(1, len(u["chunks"]))] + [(k, None)]
        todo = [(k, c) for k, u in enumerate(quads) for c in range(len(u["chunks"]))]
        ms, ws, sv, l, o = {0: m}, {}, {}, {}, {}
        first = LAG
        if prev is not None:
            ms[-1], l[-1], o[-1] = carry
            todo = [(-1, len(prev["chunks"]) - 1)] + todo
            first = LAG - 1
        for i in range(len(todo) + first):
            if i < len(ahead):
                k, c = ahead[i]
                if c is not None:
                    if k not in ws:
                        ws[k] = quads[k]["w"]()
                    sv[(k, c)] = quads[k]["chunks"][c]["qk"](ws[k])
                else:
                    nxt = quads[k + 1] if k + 1 < len(quads) else after
                    if nxt is not None:
                        ms[k + 1] = probe(nxt)
            if i < first:
                continue
            k, c = todo[i - first]
            u = prev if k < 0 else quads[k]
            if k < 0:
                pb = [p_held[j] for j in range(4)]
            else:
                p = jnp.exp2((s_probe[u["slot"]] if c == 0 else sv.pop((k, c))) - ms[k])
                l[k] = _colsum8(p) if c == 0 else l[k] + _colsum8(p)
                pb = [p[:, j * 128:(j + 1) * 128].astype(bf16) for j in range(4)]
                if hold and i - first == len(todo) - 1:
                    for j in range(4):
                        p_held[j] = pb[j]
                    continue
            oc = [_dot(u["chunks"][c]["v"](j), pb[j]) for j in range(4)]
            o[k] = oc if c == 0 else [a + b for a, b in zip(o[k], oc)]
            if c == len(u["chunks"]) - 1:
                lt = jnp.sum(l.pop(k), axis=0, keepdims=True)
                rl = 1.0 / lt
                for j, oj in enumerate(o.pop(k)):
                    u["out"](j, (oj * rl[:, j * 128:(j + 1) * 128]).astype(bf16))
                bad = jnp.where((lt <= L_MAX) & (ms[k] >= M_MIN), bad, 1.0)
        kl = len(quads) - 1
        return ms.get(len(quads)), bad, ((ms[kl], l[kl], o[kl]) if hold else None)

    def redo_with_true_max(bad, v_absmax, n_quad):
        @pl.when(jnp.logical_or(jnp.max(bad) > 0.0, jnp.logical_not(v_absmax <= V_MAX)))
        def _():
            def body(n, carry):
                w, qk, vt, out = n_quad(n)

                def pass1(c, mrun):
                    s = qk(w, _tile(c))
                    s_all[pl.ds(_tile(c), 128), :] = s
                    return jnp.maximum(mrun, _colmax8(s))
                mrun = lax.fori_loop(0, NT, pass1, jnp.full((8, 512), -jnp.inf, f32))
                m = jnp.max(mrun, axis=0, keepdims=True)

                def pass2(c, lo):
                    p = jnp.exp2(s_all[pl.ds(_tile(c), 128), :] - m)
                    oc = jnp.concatenate(
                        [_dot(vt(j, _tile(c)), p[:, j * 128:(j + 1) * 128].astype(bf16)) for j in range(4)], axis=1)
                    return lo[0] + _colsum8(p), lo[1] + oc
                l, o = lax.fori_loop(0, NT, pass2, (jnp.zeros((8, 512), f32), jnp.zeros((DH, 512), f32)))
                o = o * (1.0 / jnp.sum(l, axis=0, keepdims=True))
                for j in range(4):
                    out(j, o[:, j * 128:(j + 1) * 128].astype(bf16))
                return carry
            lax.fori_loop(0, NQ, body, 0)

    def head_rows(gl, j):
        return pl.ds(gl + j * DH if isinstance(gl, int) else pl.multiple_of(gl + j * DH, DH), DH)

    def store_head(gl, tq, j, val):
        ot[head_rows(gl, j), pl.ds(tq, 128)] = val

    def stationary(gl, tq, diagonal):
        blocks = []
        for j in range(4):
            above = j * DH if diagonal else 0
            parts = [jnp.zeros((above, 128), bf16)] if above else []
            parts.append(qt[head_rows(gl, j), pl.ds(tq, 128)])
            if above + DH < 128:
                parts.append(jnp.zeros((128 - above - DH, 128), bf16))
            blocks.append(jnp.concatenate(parts, axis=0))
        return jnp.concatenate(blocks, axis=1)

    no_flag = jnp.zeros((1, 512), f32)

    def a_quad(n, slot):
        tq, gl = _tile(n // NG), _tile(n % NG)

        def chunk(c):
            keys = pl.ds(c * 128, 128)
            return dict(qk=lambda w: _dot(kpad[keys, :], w), v=lambda j: vta[:, keys])
        return dict(w=lambda: stationary(gl, tq, False), chunks=[chunk(c) for c in range(NT)], slot=slot,
                    out=functools.partial(store_head, gl, tq))

    p_held[...] = jnp.zeros(p_held.shape, bf16)
    m = probe(a_quad(0, 0))
    held = (no_flag, jnp.ones((8, 512), f32), [jnp.zeros((DH, 128), f32)] * 4)
    for cp in (cp_woa, cp_xb, cp_wqkv, cp_wob):
        cp.start()

    def a_trip(i, carry):
        n = i * A_STEP
        m, bad, held = carry
        return stream([a_quad(n + k, k % 2) for k in range(A_STEP)], m, bad,
                      a_quad(jnp.minimum(n + A_STEP, NQ - 1), 0),
                      prev=a_quad(jnp.maximum(n - 1, 0), 1), carry=held, hold=True)

    m, bad, held = lax.fori_loop(0, NQ // A_STEP, a_trip, (m, no_flag, held))
    _, bad, _ = stream([], m, bad, None, prev=a_quad(NQ - 1, 1), carry=held)

    def a_exact(n):
        tq, gl = _tile(n // NG), _tile(n % NG)
        return (stationary(gl, tq, False), lambda w, k0: _dot(kpad[pl.ds(k0, 128), :], w),
                lambda j, k0: vta[:, pl.ds(k0, 128)], functools.partial(store_head, gl, tq))

    redo_with_true_max(bad, jnp.max(jnp.abs(vta[...].astype(f32))), a_exact)

    def out_copy(part, i):
        a, n = OUT_BLOCKS[i]
        return pltpu.make_async_copy(ostage.at[part, pl.ds(a, n), :], out_hbm.at[0, pl.ds(a, n), pl.ds(part * D, D)],
                                     out_sem.at[part * len(OUT_BLOCKS) + i])

    def out_proj(part, wo):
        for i, (a, n) in enumerate(OUT_BLOCKS):
            y = lax.dot_general(ot[:, pl.ds(a, n)], wo[...], TN_DIMS, preferred_element_type=f32)
            ostage[part, pl.ds(a, n), :] = y.astype(bf16)
            out_copy(part, i).start()

    cp_woa.wait()
    cp_xb.wait()
    cp_wqkv.wait()
    cp_wob.wait()
    out_proj(0, woa)

    def b_proj(r, vmax):
        rows = pl.ds(pl.multiple_of(r * BR, BR), BR)
        x = xb[rows, :]
        qt[:, rows] = (_dot(x, wqkv[:, 0:D]) * QSCALE).astype(bf16).T
        kb[rows, :] = _dot(x, wqkv[:, D:2 * D]).astype(bf16)
        v = _dot(x, wqkv[:, 2 * D:3 * D])
        vtb[:, rows] = v.astype(bf16).T
        return jnp.maximum(vmax, _colmax8(jnp.abs(v)))

    vb_absmax = jnp.max(lax.fori_loop(0, S // BR, b_proj, jnp.zeros((8, D), f32)))

    def b_quad(t, g):
        gl, tq = g * 128, t * 128

        def chunk(back, mask):
            keys = pl.ds(tq - back * 128, 128)

            def qk(w):
                s = _dot(kb[keys, gl:gl + 128], w)
                return s if mask is None else s + jnp.concatenate([bias[mask]] * 4, axis=1)
            return dict(qk=qk, v=lambda j: vtb[head_rows(gl, j), keys])
        chunks = [chunk(1, None), chunk(2, 0), chunk(0, 1)]
        if t < 2:
            chunks = chunks[2:] if t == 0 else [chunks[0], chunks[2]]
        return dict(w=lambda: stationary(gl, tq, True), chunks=chunks, slot=g % 4,
                    out=functools.partial(store_head, gl, tq))

    _, bad, _ = stream([b_quad(t, g) for t in range(NT) for g in range(NG)], probe(b_quad(0, 0)), no_flag, None)

    def b_exact(n):
        tq, gl = _tile(n // NG), _tile(n % NG)
        lane_head = lax.broadcasted_iota(jnp.int32, (128, 128), 0) // DH
        q = qt[pl.ds(gl, 128), pl.ds(tq, 128)].astype(f32)
        w = jnp.concatenate([jnp.where(lane_head == j, q, 0.0).astype(bf16) for j in range(4)], axis=1)
        qpos = tq + lax.broadcasted_iota(jnp.int32, (128, 512), 1) % 128

        def qk(w, k0):
            dist = qpos - (k0 + lax.broadcasted_iota(jnp.int32, (128, 512), 0))
            s = _dot(kb[pl.ds(k0, 128), pl.ds(gl, 128)], w)
            return jnp.where((dist >= 0) & (dist < WIN), s, MASKED)
        return w, qk, lambda j, k0: vtb[head_rows(gl, j), pl.ds(k0, 128)], functools.partial(store_head, gl, tq)

    redo_with_true_max(bad, vb_absmax, b_exact)

    out_proj(1, wob)
    for part in range(2):
        for i in range(len(OUT_BLOCKS)):
            out_copy(part, i).wait()


@jax.jit
def pallas_concat_heads__grouped_kv_mqa__sliding_block__prompt_kernel(
    A_x: jax.Array,
    A_wq: jax.Array,
    A_wk: jax.Array,
    A_wv: jax.Array,
    A_wo: jax.Array,
    B_x: jax.Array,
    B_wqkv: jax.Array,
    B_wo: jax.Array,
):
    hbm = pl.BlockSpec(memory_space=pl.ANY)
    vmem = pltpu.VMEM
    return pl.pallas_call(
        _kernel,
        in_specs=[hbm] * 8,
        out_specs=hbm,
        out_shape=jax.ShapeDtypeStruct((1, S, 2 * D), bf16),
        scratch_shapes=[
            vmem((S, D), bf16), vmem((D, D), bf16), vmem((DH, D), bf16), vmem((DH, D), bf16), vmem((D, D), bf16),
            vmem((S, D), bf16), vmem((D, 3 * D), bf16), vmem((D, D), bf16),
            vmem((D, S), bf16),
            vmem((S, 128), bf16),
            vmem((DH, S), bf16),
            vmem((S, D), bf16),
            vmem((D, S), bf16),
            vmem((D, S), bf16),
            vmem((4, 128, 512), f32),
            vmem((4, 128, 128), bf16),
            vmem((S, 512), f32),
            vmem((2, 128, 128), f32),
            vmem((2, S, D), bf16),
            pltpu.SemaphoreType.DMA((len(X_BLOCKS) + len(WQ_BLOCKS) + 6,)),
            pltpu.SemaphoreType.DMA((2 * len(OUT_BLOCKS),)),
        ],
        compiler_params=pltpu.CompilerParams(vmem_limit_bytes=100 * 2**20,
                                             flags={"XLA_TPU_RESCHEDULE_DMA_DONES": True}),
    )(A_x, A_wq, A_wk.T, A_wv.T, A_wo, B_x, B_wqkv, B_wo)
```
